```python
import jax
import jax.numpy as jnp

def _softmax(x, axis=-1):
    return jax.nn.softmax(x, axis=axis)
def _gelu(x):
    return jax.nn.gelu(x, approximate=True)
def _silu(x):
    return jax.nn.silu(x)
def _sigmoid(x):
    return jax.nn.sigmoid(x)
def _layernorm(x, axis=-1, eps=1e-5):
    m = jnp.mean(x, axis=axis, keepdims=True)
    v = jnp.var(x, axis=axis, keepdims=True)
    return (x - m) / jnp.sqrt(v + eps)
def _scatter_add(tgt, idx, src, axis=0):
    return tgt.at[idx].add(src)
def _segment_sum(src, seg, n):
    return jax.ops.segment_sum(src, seg, n)
class _Rng:
    def __init__(self, key):
        self._k = key
    def _next(self):
        self._k, sub = jax.random.split(self._k)
        return sub
    def normal(self, shape):
        return jax.random.normal(self._next(), shape, dtype=jnp.bfloat16)
    def randint(self, lo, hi, shape):
        return jax.random.randint(self._next(), shape, lo, hi, dtype=jnp.int32)
    def uniform(self, shape, lo=0.0, hi=1.0):
        return jax.random.uniform(self._next(), shape, jnp.bfloat16, lo, hi)
    def permutation(self, n):
        return jax.random.permutation(self._next(), n)


kernel_name = 'gated_mix__sliding_block_cached__glu_gated_swiglu__decode'

def setup_inputs():
    _rng = _Rng(jax.random.key(int.from_bytes(__import__("os").urandom(4), "little")))
    _w = (lambda a: (lambda t: t.astype(jnp.bfloat16) if jnp.issubdtype(t.dtype, jnp.floating) else t)(jnp.asarray(a)))
    def _A_setup():
        B, Sq, D = 1, 1, 640
        Hq, Hkv, Sk, Dh = 32, 32, 32768, 192
        assert Hq % Hkv == 0, (Hq, Hkv)
        return {
            "x": _w((lambda *s: _rng.normal(s) * 0.05)(B, Sq, D)),
            "k_cache": _w((lambda *s: _rng.normal(s) * 0.05)(B, Hkv, Sk, Dh)),
            "v_cache": _w((lambda *s: _rng.normal(s) * 0.05)(B, Hkv, Sk, Dh)),
            "wq": _w((lambda *s: _rng.normal(s) * 0.05)(D, Hq * Dh) * (D ** -0.5)),
            "wo": _w((lambda *s: _rng.normal(s) * 0.05)(Hq * Dh, D) * ((Hq * Dh) ** -0.5)),
        }
    _A_in = _A_setup()

    def _B_setup():
        B, S, D, F = 1, 1, 640, 1536
        return {
            "x": _w((lambda *s: _rng.normal(s) * 0.05)(B, S, D)),
            "w1": _w((lambda *s: _rng.normal(s) * 0.05)(D, F) * (2.0 / D) ** 0.5),
            "w3": _w((lambda *s: _rng.normal(s) * 0.05)(D, F) * (2.0 / D) ** 0.5),
            "w2": _w((lambda *s: _rng.normal(s) * 0.05)(F, D) * (2.0 / F) ** 0.5),
        }
    _B_in = _B_setup()

    return {
        "A_x": _A_in["x"],
        "A_k_cache": _A_in["k_cache"],
        "A_v_cache": _A_in["v_cache"],
        "A_wq": _A_in["wq"],
        "A_wo": _A_in["wo"],
        "B_x": _B_in["x"],
        "B_w1": _B_in["w1"],
        "B_w3": _B_in["w3"],
        "B_w2": _B_in["w2"],
        "gate_w": _w((lambda *s: _rng.normal(s) * 0.05)(640)),
    }

def reference(A_x, A_k_cache, A_v_cache, A_wq, A_wo, B_x, B_w1, B_w3, B_w2, gate_w):
    def _A_ref(x, k_cache, v_cache, wq, wo):
        B, Sq, D = x.shape
        Hq, Dh = 32, 192
        Hkv, Sk = k_cache.shape[1], k_cache.shape[2]
        W = min(4096, max(256, Sk // 4))
        rep = Hq // Hkv
        q = (lambda x, *d: x.transpose(*d))((x @ wq).reshape(B, Sq, Hq, Dh), 0, 2, 1, 3)
        k = jnp.repeat(k_cache[:, :, Sk - W:, :], rep, axis=1)
        v = jnp.repeat(v_cache[:, :, Sk - W:, :], rep, axis=1)
        scores = jnp.einsum("bhqd,bhkd->bhqk", q, k) * (Dh ** -0.5)
        p = _softmax(scores, axis=-1)
        o = jnp.einsum("bhqk,bhkd->bhqd", p, v)
        return (lambda x, *d: x.transpose(*d))(o, 0, 2, 1, 3).reshape(B, Sq, Hq * Dh) @ wo

    def _B_ref(x, w1, w3, w2):
        gate = jnp.einsum("bsd,df->bsf", x, w1)
        up = jnp.einsum("bsd,df->bsf", x, w3)
        h = _silu(gate) * up
        out = jnp.einsum("bsf,fd->bsd", h, w2)
        return out

    x = A_x
    g = _sigmoid((x * gate_w).sum(-1, keepdims=True))
    a = _A_ref(x, A_k_cache, A_v_cache, A_wq, A_wo)
    b = _B_ref(x, B_w1, B_w3, B_w2)
    return g * a + (1 - g) * b
```

```python
import functools

import jax
import jax.numpy as jnp
from jax import lax
import jax.experimental.pallas as pl
import jax.experimental.pallas.tpu as pltpu

_F32 = jnp.float32
_BF16 = jnp.bfloat16

_UCOLS = 512
_STRIDE = 64
_EV = 8
_EV0 = 2
_LEAD0 = 9
_LEAD1 = 14
_TAIL = (128, 64, 32, 16)
_QK_COLS = 256
_PV_ROWS = 16


def _tiles(w):
    R, C = w.shape
    return w.reshape(R // 8, 8, C // 128, 128).transpose(0, 2, 1, 3).reshape(R * C // 128, 128)


def _strided(*lists):
    return [l[u] for q in range(_STRIDE) for l in lists for u in range(q, len(l), _STRIDE)]


def _tree_sum(parts):
    while len(parts) > 1:
        parts = [parts[i] + parts[i + 1] if i + 1 < len(parts) else parts[i]
                 for i in range(0, len(parts), 2)]
    return parts[0]


def _fold_rows(p):
    return _tree_sum([p[i:i + 8] for i in range(0, p.shape[0], 8)])


def _fold_cols(p):
    return _tree_sum([p[:, i:i + 128] for i in range(0, p.shape[1], 128)])


def _to_column(row, i0, n):
    sel = (lax.broadcasted_iota(jnp.int32, (n, 128), 1)
           == lax.broadcasted_iota(jnp.int32, (n, 128), 0) + i0)
    return jnp.broadcast_to(jnp.sum(jnp.where(sel, row, 0.0), axis=-1, keepdims=True), (n, 128))


def _aligned(i, n):
    return i if isinstance(i, int) else pl.multiple_of(i, n)


@jax.jit
def pallas_gated_mix__sliding_block_cached__glu_gated_swiglu__decode_kernel(
    A_x: jax.Array,
    A_k_cache: jax.Array,
    A_v_cache: jax.Array,
    A_wq: jax.Array,
    A_wo: jax.Array,
    B_x: jax.Array,
    B_w1: jax.Array,
    B_w3: jax.Array,
    B_w2: jax.Array,
    gate_w: jax.Array,
):
    del B_x
    B, Sq, D = A_x.shape
    _, H, SK, DH = A_k_cache.shape
    F = B_w1.shape[1]
    W = min(4096, max(256, SK // 4))
    assert B == 1 and Sq == 1 and A_wq.shape[1] == H * DH
    scale = DH ** -0.5
    NC = D // 128
    NB = DH // 8 // _EV
    NE = NB * (W // _UCOLS)
    NSEM = len(_TAIL)
    assert DH % (8 * _EV) == 0 and W % _UCOLS == 0 and _LEAD0 <= _LEAD1 <= NE and NSEM > 2
    assert DH % _PV_ROWS == 0 and 128 % _PV_ROWS == 0 and F % (16 * H) == 0
    assert sum(_TAIL) * 4 == F // 8 * NC

    kT = jnp.swapaxes(A_k_cache, 2, 3).reshape(H * DH, SK)
    vT = jnp.swapaxes(A_v_cache, 2, 3).reshape(H * DH, SK)

    def kernel(x_ref, k_ref, v_ref, wq_ref, wo_ref, w1_ref, w3_ref, w2_ref, gw_ref, o_ref,
               kvbuf, wq_b, wo_b, w1_b, w3_b, w2_b, x_b, gw_b,
               xcol, qcol, hcol, qrow, hrow, s_s, sem):

        def kv_event(m, h, e):
            c, b = divmod(e, NB)
            src = v_ref if m else k_ref
            out = []
            for u0, nu in ((0, _EV - _EV0), (_EV - _EV0, _EV0)):
                r = (b * _EV + u0) * 8
                out.append([(
                    src.at[pl.ds(_aligned(h * DH + r, 8), nu * 8), pl.ds(SK - W + c * _UCOLS, _UCOLS)],
                    kvbuf.at[(h % 2) * 2 + m, pl.ds(r, nu * 8), pl.ds(c * _UCOLS, _UCOLS)],
                    m)])
            return out

        def units(src, dst):
            R, C = src.shape
            if C == 128:
                at = [(pl.ds(r, 32), pl.ds(0, 128)) for r in range(0, R, 32)]
            else:
                at = [(pl.ds(r, 8), pl.ds(c, _UCOLS))
                      for r in range(0, R, 8) for c in range(0, C, _UCOLS)]
            return [(src.at[i], dst.at[i]) for i in at]

        stream = []
        gsem = []
        gend = []

        def add_group(events, s):
            stream.extend((e, len(gsem)) for e in events)
            gsem.append(s)
            gend.append(len(stream))

        def add_units(us, s):
            events = []
            for i in range(0, len(us), _EV):
                e = [(a, b, s) for a, b in us[i:i + _EV]]
                events.append(lambda e=e: (e[:_EV - _EV0], e[_EV - _EV0:]))
            add_group(events, s)

        add_units(_strided(units(wq_ref, wq_b), units(w1_ref, w1_b), units(w3_ref, w3_b)), 0)
        add_units(_strided(units(wo_ref, wo_b)), 1)
        P = len(stream)
        for h in range(H):
            for m in (0, 1):
                add_group([functools.partial(kv_event, m, h, e) for e in range(NE)], m)
        u_w2 = units(w2_ref, w2_b)
        order = _strided(list(range(len(u_w2))))
        tail = []
        for t, n in enumerate(_TAIL):
            us, order = order[:n], order[n:]
            add_units([u_w2[u] for u in us], t)
            tail.append((us, len(stream)))
        NTOT = len(stream)
        gfree = [max([0] + [gend[p] for p in range(g) if gsem[p] == gsem[g]]) for g in range(len(gsem))]

        def start(copies, priority):
            for a, b, s in copies:
                pltpu.make_async_copy(a, b, sem.at[s]).start(priority=priority)

        def wait(copies):
            for a, b, s in copies:
                pltpu.make_async_copy(a, b, sem.at[s]).wait()

        pos = {0: 0, 1: 0, "waited": 0}

        def wait_until(n):
            while pos["waited"] < n:
                i = pos["waited"]
                assert i < pos[0] and i < pos[1]
                p1, p0 = stream[i][0]()
                wait(p1 + p0)
                pos["waited"] = i + 1
                for p, lead in ((0, _LEAD0), (1, _LEAD1)):
                    while (pos[p] < min(NTOT, i + 1 + lead)
                           and gfree[stream[pos[p]][1]] <= i + 1):
                        start(stream[pos[p]][0]()[1 - p], p)
                        pos[p] += 1

        def wait_with_tasks(n_end, tasks):
            n0 = pos["waited"]
            for i, task in enumerate(tasks):
                wait_until(n0 + (n_end - n0) * (i + 1) // (len(tasks) + 1))
                task()
            wait_until(n_end)

        for i in range(_LEAD1):
            p1, p0 = stream[i][0]()
            start(p1, 1)
            if i < _LEAD0:
                start(p0, 0)
        pos[0], pos[1] = _LEAD0, _LEAD1
        small = [(x_ref, x_b, NSEM - 1), (gw_ref, gw_b, NSEM - 1)]
        start(small, 1)
        wait_until(_LEAD1 + 2)
        wait(small)

        x = x_b[0].astype(_F32)
        gw = gw_b[...].reshape(1, D).astype(_F32)
        gate = jax.nn.sigmoid(jnp.sum(x * gw, axis=-1, keepdims=True))

        def x_task(r):
            n = r // 128 * 128
            xcol[r:r + 32] = _to_column(x[:, n:n + 128], r - n, 32)

        wait_with_tasks(gend[0], [functools.partial(x_task, r) for r in range(0, D, 32)])

        tmp = {}

        def matvec_tasks(w_b, j, done):
            def half(r):
                return _fold_rows(w_b[r:r + D // 2, j * 128:(j + 1) * 128].astype(_F32)
                                  * xcol[r:r + D // 2])

            def first():
                tmp["half"] = half(0)

            def second():
                done(j, jnp.sum(tmp["half"] + half(D // 2), axis=0, keepdims=True))

            return [first, second]

        def put_q(j, r):
            qrow[j:j + 1] = r * scale

        def put_gate(j, r):
            tmp["silu"] = r * jax.nn.sigmoid(r)

        def put_h(j, r):
            hrow[j:j + 1] = tmp["silu"] * r * (1.0 - gate)

        tasks = []
        for j in range(H * DH // 128):
            tasks += matvec_tasks(wq_b, j, put_q)
        for j in range(F // 128):
            tasks += matvec_tasks(w1_b, j, put_gate) + matvec_tasks(w3_b, j, put_h)
        wait_with_tasks(P, tasks)

        def column(rows_ref, i0, n):
            if isinstance(i0, int):
                return _to_column(rows_ref[i0 // 128:i0 // 128 + 1], i0 % 128, n)
            return _to_column(rows_ref[pl.ds(lax.shift_right_logical(i0, 7), 1), :], i0 & 127, n)

        def q_task(h, r):
            qcol[r:r + _PV_ROWS] = column(qrow, h * DH + r, _PV_ROWS)

        wait_with_tasks(P + NE, [functools.partial(q_task, 0, r) for r in range(0, DH, _PV_ROWS)])

        def add_tiles(acc, w, t0, coef):
            acc = list(acc)
            for i in range(w.shape[0] // 8):
                rb, n = divmod(t0 + i, NC)
                acc[n] = acc[n] + w[i * 8:(i + 1) * 8] * coef(rb)
            return acc

        def head(h, acc, last):
            def event(j):
                if last:
                    wait_until(min(P + NE + 2 * NE * h + j + 1, tail[0][1]))
                    return

                def copies(j):
                    k = j // NE + 1
                    return kv_event(k % 2, h + k // 2, j % NE)

                p1, p0 = copies(j)
                wait(p1 + p0)
                start(copies(j + _LEAD0)[1], 0)
                start(copies(j + _LEAD1)[0], 1)

            kb = kvbuf.at[(h % 2) * 2]
            vb = kvbuf.at[(h % 2) * 2 + 1]
            c = {"acc": acc}

            def scores(n0):
                q = qcol[...]
                k = kb[:, n0:n0 + _QK_COLS].astype(_F32)
                for n in range(0, _QK_COLS, 128):
                    s = jnp.sum(_fold_rows(k[:, n:n + 128] * q), axis=0, keepdims=True)
                    s = jnp.broadcast_to(s, (8, 128))
                    s_s[:, n0 + n:n0 + n + 128] = s
                    c["max"] = jnp.maximum(c["max"], s) if "max" in c else s

            def row_max():
                c["max"] = jnp.max(c["max"], axis=-1, keepdims=True)
                for r in range(0, F // H, 16):
                    i0 = h * (F // H) + r
                    hcol[pl.ds(_aligned(i0, 16), 16)] = column(hrow, i0, 16)

            def exps():
                e = jnp.exp(s_s[...] - c["max"])
                s_s[...] = e
                c["sum"] = _fold_cols(e)

            def row_sum():
                c["inv"] = 1.0 / jnp.sum(c["sum"], axis=-1, keepdims=True)

            npv = DH // _PV_ROWS

            def output(i):
                if i >= 2:
                    o = c.pop(("o", i - 2))
                    r = _aligned((h * DH + (i - 2) * _PV_ROWS) * NC, 16)
                    w = wo_b[pl.ds(r, _PV_ROWS * NC), :].astype(_F32)
                    c["acc"] = add_tiles(c["acc"], w, 0, lambda rb: o[rb])
                if 1 <= i <= npv:
                    c["o", i - 1] = [jnp.sum(t, axis=-1, keepdims=True) * c["inv"]
                                     for t in c.pop(("pv", i - 1))]
                    if not last:
                        q_task(h + 1, (i - 1) * _PV_ROWS)
                if i < npv:
                    v = vb[i * _PV_ROWS:(i + 1) * _PV_ROWS, :].astype(_F32)
                    p = s_s[...]
                    c["pv", i] = [_fold_cols(v[r:r + 8] * p) for r in range(0, _PV_ROWS, 8)]

            halves = (
                [functools.partial(scores, n0) for n0 in range(0, W, _QK_COLS)]
                + [row_max, exps, row_sum],
                [functools.partial(output, i) for i in range(npv + 2)],
            )
            for half, tasks in enumerate(halves):
                span = min(NE, len(tasks)) if last and half else NE
                for j in range(NE):
                    for i, task in enumerate(tasks):
                        if i * span // len(tasks) == j:
                            task()
                    event(half * NE + j)
            return tuple(c["acc"])

        assert pos["waited"] == P + NE
        assert pos[0] == P + NE + _LEAD0 and pos[1] == P + NE + _LEAD1
        acc = tuple(jnp.zeros((8, 128), _F32) for _ in range(NC))
        acc = lax.fori_loop(0, H - 1, lambda h, a: head(h, a, False), acc)
        for k in (0, 1, "waited"):
            pos[k] += (H - 1) * 2 * NE
        acc = head(H - 1, acc, True)

        acc = [a * gate for a in acc]

        def add_w2(acc, us):
            for u in us:
                acc = add_tiles(acc, w2_b[u * 32:(u + 1) * 32].astype(_F32), u * 4,
                                lambda rb: hcol[rb * 8:(rb + 1) * 8])
            return acc

        wait_until(tail[0][1])
        for (us, end), (_, end_next) in zip(tail[:-1], tail[1:]):
            n = end_next - end
            for j in range(n):
                acc = add_w2(acc, us[len(us) * j // n:len(us) * (j + 1) // n])
                wait_until(end + j + 1)
        assert pos["waited"] == pos[0] == pos[1] == NTOT
        acc = add_w2(acc, tail[-1][0])
        out = jnp.concatenate([jnp.sum(a, axis=0, keepdims=True) for a in acc], axis=1)
        o_ref[0] = out.astype(o_ref.dtype)

    hbm = pl.BlockSpec(memory_space=pl.ANY)
    return pl.pallas_call(
        kernel,
        out_shape=jax.ShapeDtypeStruct((B, Sq, D), A_x.dtype),
        in_specs=[hbm] * 9,
        out_specs=pl.BlockSpec(memory_space=pltpu.VMEM),
        scratch_shapes=[
            pltpu.VMEM((4, DH, W), _BF16),
            pltpu.VMEM((D, H * DH), _BF16),
            pltpu.VMEM((H * DH * NC, 128), _BF16),
            pltpu.VMEM((D, F), _BF16),
            pltpu.VMEM((D, F), _BF16),
            pltpu.VMEM((F * NC, 128), _BF16),
            pltpu.VMEM((1, 1, D), _BF16),
            pltpu.VMEM((D,), _BF16),
            pltpu.VMEM((D, 128), _F32),
            pltpu.VMEM((DH, 128), _F32),
            pltpu.VMEM((F, 128), _F32),
            pltpu.VMEM((H * DH // 128, 128), _F32),
            pltpu.VMEM((F // 128, 128), _F32),
            pltpu.VMEM((8, W), _F32),
            pltpu.SemaphoreType.DMA((NSEM,)),
        ],
        compiler_params=pltpu.CompilerParams(
            vmem_limit_bytes=48 * 1024 * 1024,
            disable_bounds_checks=True,
            disable_semaphore_checks=True,
        ),
    )(A_x, kT, vT, A_wq, _tiles(A_wo), B_w1, B_w3, _tiles(B_w2), gate_w)
```

```python
import functools

import jax
import jax.numpy as jnp
from jax import lax
import jax.experimental.pallas as pl
import jax.experimental.pallas.tpu as pltpu

_F32 = jnp.float32
_BF16 = jnp.bfloat16

_UCOLS = 512
_STRIDE = 64
_EV = 8
_EV0_KV = 1
_EV0_W = 2
_LEAD0 = 9
_LEAD1 = 14
_TAIL = (128, 56, 24, 16, 8, 8)
_QK_COLS = 256
_PV_ROWS = 16


def _tiles(w):
    R, C = w.shape
    return w.reshape(R // 8, 8, C // 128, 128).transpose(0, 2, 1, 3).reshape(R * C // 128, 128)


def _sweeps(n):
    return [q for q in range(n) if q % 4 in (0, 3)][::-1] + [q for q in range(n) if q % 4 in (1, 2)]


def _strided(*lists):
    return [l[u] for q in _sweeps(_STRIDE) for l in lists for u in range(q, len(l), _STRIDE)]


def _tree_sum(parts):
    while len(parts) > 1:
        parts = [parts[i] + parts[i + 1] if i + 1 < len(parts) else parts[i]
                 for i in range(0, len(parts), 2)]
    return parts[0]


def _fold_rows(p):
    return _tree_sum([p[i:i + 8] for i in range(0, p.shape[0], 8)])


def _fold_cols(p):
    return _tree_sum([p[:, i:i + 128] for i in range(0, p.shape[1], 128)])


def _to_column(row, i0, n):
    sel = (lax.broadcasted_iota(jnp.int32, (n, 128), 1)
           == lax.broadcasted_iota(jnp.int32, (n, 128), 0) + i0)
    return jnp.broadcast_to(jnp.sum(jnp.where(sel, row, 0.0), axis=-1, keepdims=True), (n, 128))


def _aligned(i, n):
    return i if isinstance(i, int) else pl.multiple_of(i, n)


@jax.jit
def pallas_gated_mix__sliding_block_cached__glu_gated_swiglu__decode_kernel(
    A_x: jax.Array,
    A_k_cache: jax.Array,
    A_v_cache: jax.Array,
    A_wq: jax.Array,
    A_wo: jax.Array,
    B_x: jax.Array,
    B_w1: jax.Array,
    B_w3: jax.Array,
    B_w2: jax.Array,
    gate_w: jax.Array,
):
    del B_x
    B, Sq, D = A_x.shape
    _, H, SK, DH = A_k_cache.shape
    F = B_w1.shape[1]
    W = min(4096, max(256, SK // 4))
    assert B == 1 and Sq == 1 and A_wq.shape[1] == H * DH
    scale = DH ** -0.5
    NC = D // 128
    NB = DH // 8 // _EV
    NE = NB * (W // _UCOLS)
    NSEM = len(_TAIL)
    assert DH % (8 * _EV) == 0 and W % _UCOLS == 0 and _LEAD0 <= _LEAD1 <= NE and NSEM > 2
    assert DH % _PV_ROWS == 0 and 128 % _PV_ROWS == 0 and F % (16 * H) == 0
    assert sum(_TAIL) * 4 == F // 8 * NC

    kT = jnp.swapaxes(A_k_cache, 2, 3).reshape(H * DH, SK)
    vT = jnp.swapaxes(A_v_cache, 2, 3).reshape(H * DH, SK)

    def kernel(x_ref, k_ref, v_ref, wq_ref, wo_ref, w1_ref, w3_ref, w2_ref, gw_ref, o_ref,
               kvbuf, wq_b, wo_b, w1_b, w3_b, w2_b, x_b, gw_b,
               xcol, qcol, hcol, qrow, hrow, s_s, sem):

        def kv_event(m, h, e):
            c, b = _sweeps(W // _UCOLS)[e // NB], e % NB
            src = v_ref if m else k_ref
            out = []
            for u0, nu in ((0, _EV - _EV0_KV), (_EV - _EV0_KV, _EV0_KV)):
                r = (b * _EV + u0) * 8
                out.append([(
                    src.at[pl.ds(_aligned(h * DH + r, 8), nu * 8), pl.ds(SK - W + c * _UCOLS, _UCOLS)],
                    kvbuf.at[(h % 2) * 2 + m, pl.ds(r, nu * 8), pl.ds(c * _UCOLS, _UCOLS)],
                    m)])
            return out

        def units(src, dst):
            R, C = src.shape
            if C == 128:
                at = [(pl.ds(r, 32), pl.ds(0, 128)) for r in range(0, R, 32)]
            else:
                at = [(pl.ds(r, 8), pl.ds(c, _UCOLS))
                      for r in range(0, R, 8) for c in range(0, C, _UCOLS)]
            return [(src.at[i], dst.at[i]) for i in at]

        stream = []
        gsem = []
        gend = []

        def add_group(events, s):
            stream.extend((e, len(gsem)) for e in events)
            gsem.append(s)
            gend.append(len(stream))

        def add_units(us, s):
            events = []
            for i in range(0, len(us), _EV):
                e = [(a, b, s) for a, b in us[i:i + _EV]]
                events.append(lambda e=e: (e[:_EV - _EV0_W], e[_EV - _EV0_W:]))
            add_group(events, s)

        add_units(_strided(units(wq_ref, wq_b), units(w1_ref, w1_b), units(w3_ref, w3_b)), 0)
        add_units(_strided(units(wo_ref, wo_b)), 1)
        P = len(stream)
        for h in range(H):
            for m in (0, 1):
                add_group([functools.partial(kv_event, m, h, e) for e in range(NE)], m)
        u_w2 = units(w2_ref, w2_b)
        order = _strided(list(range(len(u_w2))))
        tail = []
        for t, n in enumerate(_TAIL):
            us, order = order[:n], order[n:]
            add_units([u_w2[u] for u in us], t)
            tail.append((us, len(stream)))
        NTOT = len(stream)
        gfree = [max([0] + [gend[p] for p in range(g) if gsem[p] == gsem[g]]) for g in range(len(gsem))]

        def start(copies, priority):
            for a, b, s in copies:
                pltpu.make_async_copy(a, b, sem.at[s]).start(priority=priority)

        def wait(copies):
            for a, b, s in copies:
                pltpu.make_async_copy(a, b, sem.at[s]).wait()

        pos = {0: 0, 1: 0, "waited": 0}

        def wait_until(n):
            while pos["waited"] < n:
                i = pos["waited"]
                assert i < pos[0] and i < pos[1]
                p1, p0 = stream[i][0]()
                wait(p1 + p0)
                pos["waited"] = i + 1
                for p, lead in ((0, _LEAD0), (1, _LEAD1)):
                    while (pos[p] < min(NTOT, i + 1 + lead)
                           and gfree[stream[pos[p]][1]] <= i + 1):
                        start(stream[pos[p]][0]()[1 - p], p)
                        pos[p] += 1

        def wait_with_tasks(n_end, tasks):
            n0 = pos["waited"]
            for i, task in enumerate(tasks):
                wait_until(n0 + (n_end - n0) * (i + 1) // (len(tasks) + 1))
                task()
            wait_until(n_end)

        for i in range(_LEAD1):
            p1, p0 = stream[i][0]()
            start(p1, 1)
            if i < _LEAD0:
                start(p0, 0)
        pos[0], pos[1] = _LEAD0, _LEAD1
        small = [(x_ref, x_b, NSEM - 1), (gw_ref, gw_b, NSEM - 1)]
        start(small, 1)
        wait_until(_LEAD1 + 2)
        wait(small)

        x = x_b[0].astype(_F32)
        gw = gw_b[...].reshape(1, D).astype(_F32)
        gate = jax.nn.sigmoid(jnp.sum(x * gw, axis=-1, keepdims=True))

        def x_task(r):
            n = r // 128 * 128
            xcol[r:r + 32] = _to_column(x[:, n:n + 128], r - n, 32)

        wait_with_tasks(gend[0], [functools.partial(x_task, r) for r in range(0, D, 32)])

        tmp = {}

        def matvec_tasks(w_b, j, done):
            def half(r):
                return _fold_rows(w_b[r:r + D // 2, j * 128:(j + 1) * 128].astype(_F32)
                                  * xcol[r:r + D // 2])

            def first():
                tmp["half"] = half(0)

            def second():
                done(j, jnp.sum(tmp["half"] + half(D // 2), axis=0, keepdims=True))

            return [first, second]

        def put_q(j, r):
            qrow[j:j + 1] = r * scale

        def put_gate(j, r):
            tmp["silu"] = r * jax.nn.sigmoid(r)

        def put_h(j, r):
            hrow[j:j + 1] = tmp["silu"] * r * (1.0 - gate)

        tasks = []
        for j in range(H * DH // 128):
            tasks += matvec_tasks(wq_b, j, put_q)
        for j in range(F // 128):
            tasks += matvec_tasks(w1_b, j, put_gate) + matvec_tasks(w3_b, j, put_h)
        wait_with_tasks(P, tasks)

        def column(rows_ref, i0, n):
            if isinstance(i0, int):
                return _to_column(rows_ref[i0 // 128:i0 // 128 + 1], i0 % 128, n)
            return _to_column(rows_ref[pl.ds(lax.shift_right_logical(i0, 7), 1), :], i0 & 127, n)

        def q_task(h, r):
            qcol[r:r + _PV_ROWS] = column(qrow, h * DH + r, _PV_ROWS)

        wait_with_tasks(P + NE, [functools.partial(q_task, 0, r) for r in range(0, DH, _PV_ROWS)])

        def add_tiles(acc, w, t0, coef):
            acc = list(acc)
            for i in range(w.shape[0] // 8):
                rb, n = divmod(t0 + i, NC)
                acc[n] = acc[n] + w[i * 8:(i + 1) * 8] * coef(rb)
            return acc

        def head(h, acc, last):
            def event(j):
                if last:
                    wait_until(min(P + NE + 2 * NE * h + j + 1, tail[0][1]))
                    return

                def copies(j):
                    k = j // NE + 1
                    return kv_event(k % 2, h + k // 2, j % NE)

                p1, p0 = copies(j)
                wait(p1 + p0)
                start(copies(j + _LEAD0)[1], 0)
                start(copies(j + _LEAD1)[0], 1)

            kb = kvbuf.at[(h % 2) * 2]
            vb = kvbuf.at[(h % 2) * 2 + 1]
            c = {"acc": acc}

            def scores(n0):
                q = qcol[...]
                k = kb[:, n0:n0 + _QK_COLS].astype(_F32)
                for n in range(0, _QK_COLS, 128):
                    s = jnp.sum(_fold_rows(k[:, n:n + 128] * q), axis=0, keepdims=True)
                    s = jnp.broadcast_to(s, (8, 128))
                    s_s[:, n0 + n:n0 + n + 128] = s
                    c["max"] = jnp.maximum(c["max"], s) if "max" in c else s

            def row_max():
                c["max"] = jnp.max(c["max"], axis=-1, keepdims=True)
                for r in range(0, F // H, 16):
                    i0 = h * (F // H) + r
                    hcol[pl.ds(_aligned(i0, 16), 16)] = column(hrow, i0, 16)

            def exps():
                e = jnp.exp(s_s[...] - c["max"])
                s_s[...] = e
                c["sum"] = _fold_cols(e)

            def row_sum():
                c["inv"] = 1.0 / jnp.sum(c["sum"], axis=-1, keepdims=True)

            npv = DH // _PV_ROWS

            def output(i):
                if i >= 2:
                    o = c.pop(("o", i - 2))
                    r = _aligned((h * DH + (i - 2) * _PV_ROWS) * NC, 16)
                    w = wo_b[pl.ds(r, _PV_ROWS * NC), :].astype(_F32)
                    c["acc"] = add_tiles(c["acc"], w, 0, lambda rb: o[rb])
                if 1 <= i <= npv:
                    c["o", i - 1] = [jnp.sum(t, axis=-1, keepdims=True) * c["inv"]
                                     for t in c.pop(("pv", i - 1))]
                    if not last:
                        q_task(h + 1, (i - 1) * _PV_ROWS)
                if i < npv:
                    v = vb[i * _PV_ROWS:(i + 1) * _PV_ROWS, :].astype(_F32)
                    p = s_s[...]
                    c["pv", i] = [_fold_cols(v[r:r + 8] * p) for r in range(0, _PV_ROWS, 8)]

            halves = (
                [functools.partial(scores, n0) for n0 in range(0, W, _QK_COLS)]
                + [row_max, exps, row_sum],
                [functools.partial(output, i) for i in range(npv + 2)],
            )
            for half, tasks in enumerate(halves):
                span = min(NE, len(tasks)) if last and half else NE
                for j in range(NE):
                    for i, task in enumerate(tasks):
                        if i * span // len(tasks) == j:
                            task()
                    event(half * NE + j)
            return tuple(c["acc"])

        assert pos["waited"] == P + NE
        assert pos[0] == P + NE + _LEAD0 and pos[1] == P + NE + _LEAD1
        acc = tuple(jnp.zeros((8, 128), _F32) for _ in range(NC))
        acc = lax.fori_loop(0, H - 1, lambda h, a: head(h, a, False), acc)
        for k in (0, 1, "waited"):
            pos[k] += (H - 1) * 2 * NE
        acc = head(H - 1, acc, True)

        acc = [a * gate for a in acc]

        def add_w2(acc, us):
            for u in us:
                acc = add_tiles(acc, w2_b[u * 32:(u + 1) * 32].astype(_F32), u * 4,
                                lambda rb: hcol[rb * 8:(rb + 1) * 8])
            return acc

        wait_until(tail[0][1])
        for (us, end), (_, end_next) in zip(tail[:-1], tail[1:]):
            n = end_next - end
            for j in range(n):
                acc = add_w2(acc, us[len(us) * j // n:len(us) * (j + 1) // n])
                wait_until(end + j + 1)
        assert pos["waited"] == pos[0] == pos[1] == NTOT
        acc = add_w2(acc, tail[-1][0])
        out = jnp.concatenate([jnp.sum(a, axis=0, keepdims=True) for a in acc], axis=1)
        o_ref[0] = out.astype(o_ref.dtype)

    hbm = pl.BlockSpec(memory_space=pl.ANY)
    return pl.pallas_call(
        kernel,
        out_shape=jax.ShapeDtypeStruct((B, Sq, D), A_x.dtype),
        in_specs=[hbm] * 9,
        out_specs=pl.BlockSpec(memory_space=pltpu.VMEM),
        scratch_shapes=[
            pltpu.VMEM((4, DH, W), _BF16),
            pltpu.VMEM((D, H * DH), _BF16),
            pltpu.VMEM((H * DH * NC, 128), _BF16),
            pltpu.VMEM((D, F), _BF16),
            pltpu.VMEM((D, F), _BF16),
            pltpu.VMEM((F * NC, 128), _BF16),
            pltpu.VMEM((1, 1, D), _BF16),
            pltpu.VMEM((D,), _BF16),
            pltpu.VMEM((D, 128), _F32),
            pltpu.VMEM((DH, 128), _F32),
            pltpu.VMEM((F, 128), _F32),
            pltpu.VMEM((H * DH // 128, 128), _F32),
            pltpu.VMEM((F // 128, 128), _F32),
            pltpu.VMEM((8, W), _F32),
            pltpu.SemaphoreType.DMA((NSEM,)),
        ],
        compiler_params=pltpu.CompilerParams(
            vmem_limit_bytes=48 * 1024 * 1024,
            disable_bounds_checks=True,
            disable_semaphore_checks=True,
        ),
    )(A_x, kT, vT, A_wq, _tiles(A_wo), B_w1, B_w3, _tiles(B_w2), gate_w)
```

```python
import functools

import jax
import jax.numpy as jnp
from jax import lax
import jax.experimental.pallas as pl
import jax.experimental.pallas.tpu as pltpu

_F32 = jnp.float32
_BF16 = jnp.bfloat16

_UCOLS = 512
_STRIDE = 64
_EV = 8
_EV0_KV = 1
_EV0_W = 2
_LEAD0 = 9
_LEAD1 = 14
_TAIL = (128, 56, 24, 16, 8, 8)
_QK_COLS = 256
_PV_ROWS = 16


def _tiles(w):
    R, C = w.shape
    return w.reshape(R // 8, 8, C // 128, 128).transpose(0, 2, 1, 3).reshape(R * C // 128, 128)


def _sweeps(n):
    return [q for q in range(n) if q % 4 in (0, 3)][::-1] + [q for q in range(n) if q % 4 in (1, 2)]


def _strided(*lists):
    return [l[u] for q in _sweeps(_STRIDE) for l in lists for u in range(q, len(l), _STRIDE)]


def _fold(p, axis, size):
    def add_parts(p, n):
        parts = [lax.slice_in_dim(p, i, i + n, axis=axis) for i in range(0, p.shape[axis], n)]
        return functools.reduce(lambda a, b: a + b, parts)

    while p.shape[axis] % (2 * size) == 0:
        p = add_parts(p, p.shape[axis] // 2)
    return add_parts(p, size)


def _fold_rows(p):
    return _fold(p, 0, 8)


def _fold_cols(p):
    return _fold(p, 1, 128)


def _to_column(row, i0, n):
    sel = (lax.broadcasted_iota(jnp.int32, (n, 128), 1)
           == lax.broadcasted_iota(jnp.int32, (n, 128), 0) + i0)
    return jnp.broadcast_to(jnp.sum(jnp.where(sel, row, 0.0), axis=-1, keepdims=True), (n, 128))


def _aligned(i, n):
    return i if isinstance(i, int) else pl.multiple_of(i, n)


@jax.jit
def pallas_gated_mix__sliding_block_cached__glu_gated_swiglu__decode_kernel(
    A_x: jax.Array,
    A_k_cache: jax.Array,
    A_v_cache: jax.Array,
    A_wq: jax.Array,
    A_wo: jax.Array,
    B_x: jax.Array,
    B_w1: jax.Array,
    B_w3: jax.Array,
    B_w2: jax.Array,
    gate_w: jax.Array,
):
    del B_x
    B, Sq, D = A_x.shape
    _, H, SK, DH = A_k_cache.shape
    F = B_w1.shape[1]
    W = min(4096, max(256, SK // 4))
    assert B == 1 and Sq == 1 and A_wq.shape[1] == H * DH
    scale = DH ** -0.5
    NC = D // 128
    NB = DH // 8 // _EV
    NE = NB * (W // _UCOLS)
    NSEM = len(_TAIL)
    assert DH % (8 * _EV) == 0 and W % _UCOLS == 0 and _LEAD0 <= _LEAD1 <= NE and NSEM > 2
    assert DH % _PV_ROWS == 0 and 128 % _PV_ROWS == 0 and F % (16 * H) == 0
    assert sum(_TAIL) * 4 == F // 8 * NC

    kT = jnp.swapaxes(A_k_cache, 2, 3).reshape(H * DH, SK)
    vT = jnp.swapaxes(A_v_cache, 2, 3).reshape(H * DH, SK)

    def kernel(x_ref, k_ref, v_ref, wq_ref, wo_ref, w1_ref, w3_ref, w2_ref, gw_ref, o_ref,
               kvbuf, wq_b, wo_b, w1_b, w3_b, w2_b, x_b, gw_b,
               xcol, qcol, hcol, qrow, hrow, s_s, sem):

        def kv_event(m, h, e):
            c, b = _sweeps(W // _UCOLS)[e // NB], e % NB
            src = v_ref if m else k_ref
            out = []
            for u0, nu in ((0, _EV - _EV0_KV), (_EV - _EV0_KV, _EV0_KV)):
                r = (b * _EV + u0) * 8
                out.append([(
                    src.at[pl.ds(_aligned(h * DH + r, 8), nu * 8), pl.ds(SK - W + c * _UCOLS, _UCOLS)],
                    kvbuf.at[(h % 2) * 2 + m, pl.ds(r, nu * 8), pl.ds(c * _UCOLS, _UCOLS)],
                    m)])
            return out

        def units(src, dst):
            R, C = src.shape
            if C == 128:
                at = [(pl.ds(r, 32), pl.ds(0, 128)) for r in range(0, R, 32)]
            else:
                at = [(pl.ds(r, 8), pl.ds(c, _UCOLS))
                      for r in range(0, R, 8) for c in range(0, C, _UCOLS)]
            return [(src.at[i], dst.at[i]) for i in at]

        stream = []
        gsem = []
        gend = []

        def add_group(events, s):
            stream.extend((e, len(gsem)) for e in events)
            gsem.append(s)
            gend.append(len(stream))

        def add_units(us, s):
            events = []
            for i in range(0, len(us), _EV):
                e = [(a, b, s) for a, b in us[i:i + _EV]]
                events.append(lambda e=e: (e[:_EV - _EV0_W], e[_EV - _EV0_W:]))
            add_group(events, s)

        add_units(_strided(units(wq_ref, wq_b), units(w1_ref, w1_b), units(w3_ref, w3_b)), 0)
        add_units(_strided(units(wo_ref, wo_b)), 1)
        P = len(stream)
        for h in range(H):
            for m in (0, 1):
                add_group([functools.partial(kv_event, m, h, e) for e in range(NE)], m)
        u_w2 = units(w2_ref, w2_b)
        order = _strided(list(range(len(u_w2))))
        tail = []
        for t, n in enumerate(_TAIL):
            us, order = order[:n], order[n:]
            add_units([u_w2[u] for u in us], t)
            tail.append((us, len(stream)))
        NTOT = len(stream)
        gfree = [max([0] + [gend[p] for p in range(g) if gsem[p] == gsem[g]]) for g in range(len(gsem))]

        def start(copies, priority):
            for a, b, s in copies:
                pltpu.make_async_copy(a, b, sem.at[s]).start(priority=priority)

        def wait(copies):
            for a, b, s in copies:
                pltpu.make_async_copy(a, b, sem.at[s]).wait()

        pos = {0: 0, 1: 0, "waited": 0}

        def wait_until(n):
            while pos["waited"] < n:
                i = pos["waited"]
                assert i < pos[0] and i < pos[1]
                p1, p0 = stream[i][0]()
                wait(p1 + p0)
                pos["waited"] = i + 1
                for p, lead in ((0, _LEAD0), (1, _LEAD1)):
                    while (pos[p] < min(NTOT, i + 1 + lead)
                           and gfree[stream[pos[p]][1]] <= i + 1):
                        start(stream[pos[p]][0]()[1 - p], p)
                        pos[p] += 1

        def wait_with_tasks(n_end, tasks):
            n0 = pos["waited"]
            for i, task in enumerate(tasks):
                wait_until(n0 + (n_end - n0) * (i + 1) // (len(tasks) + 1))
                task()
            wait_until(n_end)

        for i in range(_LEAD1):
            p1, p0 = stream[i][0]()
            start(p1, 1)
            if i < _LEAD0:
                start(p0, 0)
        pos[0], pos[1] = _LEAD0, _LEAD1
        small = [(x_ref, x_b, NSEM - 1), (gw_ref, gw_b, NSEM - 1)]
        start(small, 1)
        wait_until(_LEAD1 + 2)
        wait(small)

        x = x_b[0].astype(_F32)
        gw = gw_b[...].reshape(1, D).astype(_F32)
        gate = jax.nn.sigmoid(jnp.sum(x * gw, axis=-1, keepdims=True))

        def x_task(r):
            n = r // 128 * 128
            xcol[r:r + 32] = _to_column(x[:, n:n + 128], r - n, 32)

        wait_with_tasks(gend[0], [functools.partial(x_task, r) for r in range(0, D, 32)])

        tmp = {}

        def matvec_tasks(w_b, j, done):
            def half(r):
                return _fold_rows(w_b[r:r + D // 2, j * 128:(j + 1) * 128].astype(_F32)
                                  * xcol[r:r + D // 2])

            def first():
                tmp["half"] = half(0)

            def second():
                done(j, jnp.sum(tmp["half"] + half(D // 2), axis=0, keepdims=True))

            return [first, second]

        def put_q(j, r):
            qrow[j:j + 1] = r * scale

        def put_gate(j, r):
            tmp["silu"] = r * jax.nn.sigmoid(r)

        def put_h(j, r):
            hrow[j:j + 1] = tmp["silu"] * r * (1.0 - gate)

        tasks = []
        for j in range(H * DH // 128):
            tasks += matvec_tasks(wq_b, j, put_q)
        for j in range(F // 128):
            tasks += matvec_tasks(w1_b, j, put_gate) + matvec_tasks(w3_b, j, put_h)
        wait_with_tasks(P, tasks)

        def column(rows_ref, i0, n):
            if isinstance(i0, int):
                return _to_column(rows_ref[i0 // 128:i0 // 128 + 1], i0 % 128, n)
            return _to_column(rows_ref[pl.ds(lax.shift_right_logical(i0, 7), 1), :], i0 & 127, n)

        def q_task(h, r):
            qcol[r:r + _PV_ROWS] = column(qrow, h * DH + r, _PV_ROWS)

        wait_with_tasks(P + NE, [functools.partial(q_task, 0, r) for r in range(0, DH, _PV_ROWS)])

        def add_tiles(acc, w, t0, coef):
            acc = list(acc)
            for i in range(w.shape[0] // 8):
                rb, n = divmod(t0 + i, NC)
                acc[n] = acc[n] + w[i * 8:(i + 1) * 8] * coef(rb)
            return acc

        def head(h, acc, last):
            def event(j):
                if last:
                    wait_until(min(P + NE + 2 * NE * h + j + 1, tail[0][1]))
                    return

                def copies(j):
                    k = j // NE + 1
                    return kv_event(k % 2, h + k // 2, j % NE)

                p1, p0 = copies(j)
                wait(p1 + p0)
                start(copies(j + _LEAD0)[1], 0)
                start(copies(j + _LEAD1)[0], 1)

            kb = kvbuf.at[(h % 2) * 2]
            vb = kvbuf.at[(h % 2) * 2 + 1]
            c = {"acc": acc}

            def scores(n0):
                q = qcol[...]
                k = kb[:, n0:n0 + _QK_COLS].astype(_F32)
                for n in range(0, _QK_COLS, 128):
                    s = jnp.sum(_fold_rows(k[:, n:n + 128] * q), axis=0, keepdims=True)
                    s = jnp.broadcast_to(s, (8, 128))
                    s_s[:, n0 + n:n0 + n + 128] = s
                    c["max"] = jnp.maximum(c["max"], s) if "max" in c else s

            def row_max():
                c["max"] = jnp.max(c["max"], axis=-1, keepdims=True)
                for r in range(0, F // H, 16):
                    i0 = h * (F // H) + r
                    hcol[pl.ds(_aligned(i0, 16), 16)] = column(hrow, i0, 16)

            def exps():
                e = jnp.exp(s_s[...] - c["max"])
                s_s[...] = e
                c["sum"] = _fold_cols(e)

            def row_sum():
                c["inv"] = 1.0 / jnp.sum(c["sum"], axis=-1, keepdims=True)

            npv = DH // _PV_ROWS

            def output(i):
                if i >= 2:
                    o = c.pop(("o", i - 2))
                    r = _aligned((h * DH + (i - 2) * _PV_ROWS) * NC, 16)
                    w = wo_b[pl.ds(r, _PV_ROWS * NC), :].astype(_F32)
                    c["acc"] = add_tiles(c["acc"], w, 0, lambda rb: o[rb])
                if 1 <= i <= npv:
                    c["o", i - 1] = [jnp.sum(t, axis=-1, keepdims=True) * c["inv"]
                                     for t in c.pop(("pv", i - 1))]
                    if not last:
                        q_task(h + 1, (i - 1) * _PV_ROWS)
                if i < npv:
                    v = vb[i * _PV_ROWS:(i + 1) * _PV_ROWS, :].astype(_F32)
                    p = s_s[...]
                    c["pv", i] = [_fold_cols(v[r:r + 8] * p) for r in range(0, _PV_ROWS, 8)]

            halves = (
                [functools.partial(scores, n0) for n0 in range(0, W, _QK_COLS)]
                + [row_max, exps, row_sum],
                [functools.partial(output, i) for i in range(npv + 2)],
            )
            for half, tasks in enumerate(halves):
                span = min(NE, len(tasks)) if last and half else NE
                for j in range(NE):
                    for i, task in enumerate(tasks):
                        if i * span // len(tasks) == j:
                            task()
                    event(half * NE + j)
            return tuple(c["acc"])

        assert pos["waited"] == P + NE
        assert pos[0] == P + NE + _LEAD0 and pos[1] == P + NE + _LEAD1
        acc = tuple(jnp.zeros((8, 128), _F32) for _ in range(NC))
        acc = lax.fori_loop(0, H - 1, lambda h, a: head(h, a, False), acc)
        for k in (0, 1, "waited"):
            pos[k] += (H - 1) * 2 * NE
        acc = head(H - 1, acc, True)

        acc = [a * gate for a in acc]

        def add_w2(acc, us):
            for u in us:
                acc = add_tiles(acc, w2_b[u * 32:(u + 1) * 32].astype(_F32), u * 4,
                                lambda rb: hcol[rb * 8:(rb + 1) * 8])
            return acc

        wait_until(tail[0][1])
        for (us, end), (_, end_next) in zip(tail[:-1], tail[1:]):
            n = end_next - end
            for j in range(n):
                acc = add_w2(acc, us[len(us) * j // n:len(us) * (j + 1) // n])
                wait_until(end + j + 1)
        assert pos["waited"] == pos[0] == pos[1] == NTOT
        acc = add_w2(acc, tail[-1][0])
        out = jnp.concatenate([jnp.sum(a, axis=0, keepdims=True) for a in acc], axis=1)
        o_ref[0] = out.astype(o_ref.dtype)

    hbm = pl.BlockSpec(memory_space=pl.ANY)
    return pl.pallas_call(
        kernel,
        out_shape=jax.ShapeDtypeStruct((B, Sq, D), A_x.dtype),
        in_specs=[hbm] * 9,
        out_specs=pl.BlockSpec(memory_space=pltpu.VMEM),
        scratch_shapes=[
            pltpu.VMEM((4, DH, W), _BF16),
            pltpu.VMEM((D, H * DH), _BF16),
            pltpu.VMEM((H * DH * NC, 128), _BF16),
            pltpu.VMEM((D, F), _BF16),
            pltpu.VMEM((D, F), _BF16),
            pltpu.VMEM((F * NC, 128), _BF16),
            pltpu.VMEM((1, 1, D), _BF16),
            pltpu.VMEM((D,), _BF16),
            pltpu.VMEM((D, 128), _F32),
            pltpu.VMEM((DH, 128), _F32),
            pltpu.VMEM((F, 128), _F32),
            pltpu.VMEM((H * DH // 128, 128), _F32),
            pltpu.VMEM((F // 128, 128), _F32),
            pltpu.VMEM((8, W), _F32),
            pltpu.SemaphoreType.DMA((NSEM,)),
        ],
        compiler_params=pltpu.CompilerParams(
            vmem_limit_bytes=48 * 1024 * 1024,
            disable_bounds_checks=True,
            disable_semaphore_checks=True,
        ),
    )(A_x, kT, vT, A_wq, _tiles(A_wo), B_w1, B_w3, _tiles(B_w2), gate_w)
```
